```python
import jax
import jax.numpy as jnp

def _softmax(x, axis=-1):
    return jax.nn.softmax(x, axis=axis)

def _gelu(x):
    return jax.nn.gelu(x, approximate=True)

def _silu(x):
    return jax.nn.silu(x)

def _sigmoid(x):
    return jax.nn.sigmoid(x)

def _layernorm(x, axis=-1, eps=1e-05):
    m = jnp.mean(x, axis=axis, keepdims=True)
    v = jnp.var(x, axis=axis, keepdims=True)
    return (x - m) / jnp.sqrt(v + eps)

def _scatter_add(tgt, idx, src, axis=0):
    return tgt.at[idx].add(src)

def _segment_sum(src, seg, n):
    return jax.ops.segment_sum(src, seg, n)

class _Rng:

    def __init__(self, key):
        self._k = key

    def _next(self):
        self._k, sub = jax.random.split(self._k)
        return sub

    def normal(self, shape):
        return jax.random.normal(self._next(), shape, dtype=jnp.bfloat16)

    def randint(self, lo, hi, shape):
        return jax.random.randint(self._next(), shape, lo, hi, dtype=jnp.int32)

    def uniform(self, shape, lo=0.0, hi=1.0):
        return jax.random.uniform(self._next(), shape, jnp.bfloat16, lo, hi)

    def permutation(self, n):
        return jax.random.permutation(self._next(), n)
kernel_name = 'adaLN_cond__mha_block_cached__moe_arch_mod__decode'

def setup_inputs():
    _rng = _Rng(jax.random.key(int.from_bytes(__import__("os").urandom(4), "little")))
    _w = lambda a: (lambda t: t.astype(jnp.bfloat16) if jnp.issubdtype(t.dtype, jnp.floating) else t)(jnp.asarray(a))

    def _A_setup():
        B, Sq, D = (4, 1, 448)
        H, Sk, Dh = (16, 16384, 256)
        return {'x': _w((lambda *s: _rng.normal(s) * 0.05)(B, Sq, D)), 'k_cache': _w((lambda *s: _rng.normal(s) * 0.05)(B, H, Sk, Dh)), 'v_cache': _w((lambda *s: _rng.normal(s) * 0.05)(B, H, Sk, Dh)), 'wq': _w((lambda *s: _rng.normal(s) * 0.05)(D, H * Dh) * D ** (-0.5)), 'wo': _w((lambda *s: _rng.normal(s) * 0.05)(H * Dh, D) * (H * Dh) ** (-0.5))}
    _A_in = _A_setup()

    def _B_setup():
        B, S, D, F, C = (4, 1, 448, 1792, 1)
        return {'x': _w((lambda *s: _rng.normal(s) * 0.05)(B, S, D)), 'w_r': _w((lambda *s: _rng.normal(s) * 0.05)(D)), 'w_gate': _w((lambda *s: _rng.normal(s) * 0.05)(D, F)), 'w_up': _w((lambda *s: _rng.normal(s) * 0.05)(D, F)), 'w_down': _w((lambda *s: _rng.normal(s) * 0.05)(F, D))}
    _B_in = _B_setup()
    return {'A_x': _A_in['x'], 'A_k_cache': _A_in['k_cache'], 'A_v_cache': _A_in['v_cache'], 'A_wq': _A_in['wq'], 'A_wo': _A_in['wo'], 'B_x': _B_in['x'], 'B_w_r': _B_in['w_r'], 'B_w_gate': _B_in['w_gate'], 'B_w_up': _B_in['w_up'], 'B_w_down': _B_in['w_down'], 'c': _w((lambda *s: _rng.normal(s) * 0.05)(4, 448)), 'w_mod': _w((lambda *s: _rng.normal(s) * 0.05)(448, 6 * 448) * 448 ** (-0.5))}

def reference(A_x, A_k_cache, A_v_cache, A_wq, A_wo, B_x, B_w_r, B_w_gate, B_w_up, B_w_down, c, w_mod):

    def _A_ref(x, k_cache, v_cache, wq, wo):
        B, Sq, D = x.shape
        H, Dh = (16, 256)
        q = (lambda x, *d: x.transpose(*d))((x @ wq).reshape(B, Sq, H, Dh), 0, 2, 1, 3)
        scores = jnp.einsum('bhqd,bhkd->bhqk', q, k_cache) * Dh ** (-0.5)
        p = _softmax(scores, axis=-1)
        o = jnp.einsum('bhqk,bhkd->bhqd', p, v_cache)
        return (lambda x, *d: x.transpose(*d))(o, 0, 2, 1, 3).reshape(B, Sq, H * Dh) @ wo

    def _B_ref(x, w_r, w_gate, w_up, w_down):
        B, S, D = x.shape
        C = 1
        r = x @ w_r
        idx = jnp.argsort(-r, axis=-1)[:, :C]
        idx_e = jnp.repeat(idx.reshape(B, C, 1), D, axis=2)
        x_sel = jnp.take_along_axis(x, idx_e, axis=1)
        g = _silu(x_sel @ w_gate)
        u = x_sel @ w_up
        y = g * u @ w_down
        r_sel = _sigmoid(jnp.take_along_axis(r, idx, axis=1))
        y = y * r_sel.reshape(B, C, 1)
        b_off = (jnp.arange(B) * S).reshape(B, 1)
        flat_idx = (idx + b_off).reshape(B * C)
        zero = (x * 0.0).reshape(B * S, D)
        upd = _scatter_add(zero, flat_idx, y.reshape(B * C, D), axis=0)
        return x + upd.reshape(B, S, D)
    x = A_x
    mod = (_silu(c) @ w_mod).reshape(c.shape[0], 6, 1, -1)
    sa, ca, ga, sb, cb, gb = (mod[:, 0].copy(), mod[:, 1].copy(), mod[:, 2].copy(), mod[:, 3].copy(), mod[:, 4].copy(), mod[:, 5].copy())
    h = _layernorm(x, axis=-1) * (1 + ca) + sa
    x = x + ga * _A_ref(h, A_k_cache, A_v_cache, A_wq, A_wo)
    h = _layernorm(x, axis=-1) * (1 + cb) + sb
    x = x + gb * _B_ref(h, B_w_r, B_w_gate, B_w_up, B_w_down)
    return x
```

```python
import functools

import jax
import jax.numpy as jnp
from jax import lax
import jax.experimental.pallas as pl
import jax.experimental.pallas.tpu as pltpu

_B, _D, _H, _DH, _SK, _F = 4, 448, 16, 256, 16384, 1792
_F32, _BF16 = jnp.float32, jnp.bfloat16
_NT = (((1,), (1,)), ((), ()))


def _layernorm(x):
    m = jnp.mean(x, axis=-1, keepdims=True)
    d = x - m
    v = jnp.mean(d * d, axis=-1, keepdims=True)
    return d / jnp.sqrt(v + 1e-5)


def _r(x):
    return x.astype(_BF16).astype(_F32)


def _body(x_hbm, k_hbm, v_hbm, wq_hbm, wo_hbm, wr_hbm, wg_hbm, wu_hbm, wd_hbm,
          c_hbm, wm_hbm, out_ref,
          x_v, c_v, wr_v, wm_v, wq_v, wo_v, wg_v, wu_v, wd_v,
          kbuf, vbuf, q_v, wsem, ksem, vsem, *, ch, nbuf):
    B, D, H, DH = _B, _D, _H, _DH
    nc = _SK // ch
    total = H * B * nc

    def w_copy(i):
        src, dst = ((c_hbm, c_v), (wm_hbm, wm_v), (x_hbm, x_v), (wq_hbm, wq_v),
                    (wo_hbm, wo_v), (wr_hbm, wr_v), (wg_hbm, wg_v),
                    (wu_hbm, wu_v), (wd_hbm, wd_v))[i]
        return pltpu.make_async_copy(src, dst, wsem.at[i])

    def kv_copies(t):
        h = t // (B * nc)
        b = (t // nc) % B
        c = t % nc
        slot = t % nbuf
        off = pl.multiple_of(c * ch, ch)
        kc = pltpu.make_async_copy(k_hbm.at[b, h, pl.ds(off, ch), :],
                                   kbuf.at[slot], ksem.at[slot])
        vc = pltpu.make_async_copy(v_hbm.at[b, h, pl.ds(off, ch), :],
                                   vbuf.at[slot], vsem.at[slot])
        return kc, vc

    for i in range(4):
        w_copy(i).start()
    for t in range(nbuf - 1):
        kc, vc = kv_copies(t)
        kc.start()
        vc.start()
    for i in range(4, 9):
        w_copy(i).start()

    w_copy(0).wait()
    w_copy(1).wait()
    cc = c_v[...].astype(_F32)
    sc = _r(cc * _r(jax.nn.sigmoid(cc)))
    mod = _r(jnp.dot(sc.astype(_BF16), wm_v[...], preferred_element_type=_F32))
    sa, ca, ga, sb, cb, gb = (mod[:, i * D:(i + 1) * D] for i in range(6))

    w_copy(2).wait()
    x = x_v[...].astype(_F32)
    h1 = _r(_r(_r(_layernorm(x)) * _r(1.0 + ca)) + sa)
    w_copy(3).wait()
    q = _r(jnp.dot(h1.astype(_BF16), wq_v[...], preferred_element_type=_F32))
    q_v[...] = q

    w_copy(4).wait()
    row = lax.broadcasted_iota(jnp.int32, (B, DH), 0)

    def head_body(h, attn):
        qh = q_v[:, pl.ds(pl.multiple_of(h * DH, DH), DH)].astype(_BF16)

        def batch_body(b, oh):
            def chunk_body(c, carry):
                m, l, acc = carry
                t = (h * B + b) * nc + c

                @pl.when(t + nbuf - 1 < total)
                def _():
                    kc, vc = kv_copies(t + nbuf - 1)
                    kc.start()
                    vc.start()

                kc, vc = kv_copies(t)
                slot = t % nbuf
                kc.wait()
                s = lax.dot_general(qh, kbuf[slot], (((1,), (1,)), ((), ())),
                                    preferred_element_type=_F32) * (DH ** -0.5)
                m_new = jnp.maximum(m, jnp.max(s, axis=-1, keepdims=True))
                alpha = jnp.exp(m - m_new)
                p = jnp.exp(s - m_new)
                l = alpha * l + jnp.sum(p, axis=-1, keepdims=True)
                vc.wait()
                acc = alpha * acc + jnp.dot(p.astype(_BF16), vbuf[slot],
                                            preferred_element_type=_F32)
                return m_new, l, acc

            m, l, acc = lax.fori_loop(
                0, nc, chunk_body,
                (jnp.full((B, 1), -jnp.inf, _F32), jnp.zeros((B, 1), _F32),
                 jnp.zeros((B, DH), _F32)))
            return jnp.where(row == b, acc / l, oh)

        oh = lax.fori_loop(0, B, batch_body, jnp.zeros((B, DH), _F32))
        wo_h = wo_v[:, pl.ds(pl.multiple_of(h * DH, DH), DH)]
        return attn + lax.dot_general(oh.astype(_BF16), wo_h, _NT,
                                      preferred_element_type=_F32)

    attn = lax.fori_loop(0, H, head_body, jnp.zeros((B, D), _F32))

    x1 = _r(x + _r(ga * _r(attn)))
    h2 = _r(_r(_r(_layernorm(x1)) * _r(1.0 + cb)) + sb)
    for i in range(5, 9):
        w_copy(i).wait()
    wr = wr_v[...].astype(_F32).reshape(1, D)
    r = _r(jnp.sum(h2 * wr, axis=-1, keepdims=True))
    hb = h2.astype(_BF16)
    g = _r(jnp.dot(hb, wg_v[...], preferred_element_type=_F32))
    g = _r(g * _r(jax.nn.sigmoid(g)))
    u = _r(jnp.dot(hb, wu_v[...], preferred_element_type=_F32))
    y = _r(lax.dot_general(_r(g * u).astype(_BF16), wd_v[...], _NT,
                           preferred_element_type=_F32))
    y = _r(y * _r(jax.nn.sigmoid(r)))
    moe = _r(h2 + _r(h2 * 0.0 + y))
    out_ref[...] = (x1 + _r(gb * moe)).astype(out_ref.dtype)


def _build(ch=2048, nbuf=4):
    B, D, H, DH, F = _B, _D, _H, _DH, _F
    anyspec = pl.BlockSpec(memory_space=pltpu.HBM)
    return pl.pallas_call(
        functools.partial(_body, ch=ch, nbuf=nbuf),
        in_specs=[anyspec] * 11,
        out_specs=pl.BlockSpec(memory_space=pltpu.VMEM),
        out_shape=jax.ShapeDtypeStruct((B, D), _BF16),
        scratch_shapes=[
            pltpu.VMEM((B, D), _BF16),
            pltpu.VMEM((B, D), _BF16),
            pltpu.VMEM((D,), _BF16),
            pltpu.VMEM((D, 6 * D), _BF16),
            pltpu.VMEM((D, H * DH), _BF16),
            pltpu.VMEM((D, H * DH), _BF16),
            pltpu.VMEM((D, F), _BF16),
            pltpu.VMEM((D, F), _BF16),
            pltpu.VMEM((D, F), _BF16),
            pltpu.VMEM((nbuf, ch, DH), _BF16),
            pltpu.VMEM((nbuf, ch, DH), _BF16),
            pltpu.VMEM((B, H * DH), _F32),
            pltpu.SemaphoreType.DMA((9,)),
            pltpu.SemaphoreType.DMA((nbuf,)),
            pltpu.SemaphoreType.DMA((nbuf,)),
        ],
        compiler_params=pltpu.CompilerParams(
            vmem_limit_bytes=100 * 1024 * 1024),
    )


def _run(A_x, A_k_cache, A_v_cache, A_wq, A_wo, B_w_r, B_w_gate, B_w_up,
         B_w_down, c, w_mod, **cfg):
    out = _build(**cfg)(A_x.reshape(_B, _D), A_k_cache, A_v_cache, A_wq, A_wo.T,
                        B_w_r, B_w_gate, B_w_up, B_w_down.T, c, w_mod)
    return out.reshape(_B, 1, _D)


@jax.jit
def pallas_adaLN_cond__mha_block_cached__moe_arch_mod__decode_kernel(
    A_x, A_k_cache, A_v_cache, A_wq, A_wo, B_x, B_w_r, B_w_gate, B_w_up,
    B_w_down, c, w_mod,
):
    del B_x
    return _run(A_x, A_k_cache, A_v_cache, A_wq, A_wo, B_w_r, B_w_gate, B_w_up,
                B_w_down, c, w_mod)
```

```python
import functools

import jax
import jax.numpy as jnp
from jax import lax
import jax.experimental.pallas as pl
import jax.experimental.pallas.tpu as pltpu

_B, _D, _H, _DH, _SK, _F = 4, 448, 16, 256, 16384, 1792
_F32, _BF16 = jnp.float32, jnp.bfloat16
_NT = (((1,), (1,)), ((), ()))


def _layernorm(x):
    m = jnp.mean(x, axis=-1, keepdims=True)
    d = x - m
    v = jnp.mean(d * d, axis=-1, keepdims=True)
    return d / jnp.sqrt(v + 1e-5)


def _r(x):
    return x.astype(_BF16).astype(_F32)


def _body(x_hbm, k_hbm, v_hbm, wq_hbm, wo_hbm, wr_hbm, wg_hbm, wu_hbm, wd_hbm,
          c_hbm, wm_hbm, out_ref,
          x_v, c_v, wr_v, wm_v, wq_v, wo_v, wg_v, wu_v, wd_v,
          kbuf, vbuf, q_v, wsem, ksem, vsem, *, ch, nbuf, sub, prio):
    B, D, H, DH = _B, _D, _H, _DH
    nc = _SK // ch
    total = H * B * nc

    def w_copy(i):
        src, dst = ((c_hbm, c_v), (wm_hbm, wm_v), (x_hbm, x_v), (wq_hbm, wq_v),
                    (wo_hbm, wo_v), (wr_hbm, wr_v), (wg_hbm, wg_v),
                    (wu_hbm, wu_v), (wd_hbm, wd_v))[i]
        return pltpu.make_async_copy(src, dst, wsem.at[i])

    def kv_start(t):
        h = t // (B * nc)
        b = (t // nc) % B
        slot = t % nbuf
        base = (t % nc) * ch
        n = 0
        for j in range(ch // sub):
            off = pl.multiple_of(base + j * sub, sub)
            for src, dst, sem in ((k_hbm, kbuf, ksem), (v_hbm, vbuf, vsem)):
                pltpu.make_async_copy(
                    src.at[b, h, pl.ds(off, sub), :],
                    dst.at[slot, pl.ds(j * sub, sub), :],
                    sem.at[slot]).start(priority=prio[n % len(prio)])
                n += 1

    def buf_wait(buf, sem, slot):
        pltpu.make_async_copy(buf.at[slot], buf.at[slot], sem.at[slot]).wait()

    for i in range(4):
        w_copy(i).start()
    for t in range(nbuf - 1):
        kv_start(t)
    for i in range(4, 9):
        w_copy(i).start()

    w_copy(0).wait()
    w_copy(1).wait()
    cc = c_v[...].astype(_F32)
    sc = _r(cc * _r(jax.nn.sigmoid(cc)))
    mod = _r(jnp.dot(sc.astype(_BF16), wm_v[...], preferred_element_type=_F32))
    sa, ca, ga, sb, cb, gb = (mod[:, i * D:(i + 1) * D] for i in range(6))

    w_copy(2).wait()
    x = x_v[...].astype(_F32)
    h1 = _r(_r(_r(_layernorm(x)) * _r(1.0 + ca)) + sa)
    w_copy(3).wait()
    q = _r(jnp.dot(h1.astype(_BF16), wq_v[...], preferred_element_type=_F32))
    q_v[...] = q

    w_copy(4).wait()
    row = lax.broadcasted_iota(jnp.int32, (B, DH), 0)

    def head_body(h, attn):
        qh = q_v[:, pl.ds(pl.multiple_of(h * DH, DH), DH)].astype(_BF16)

        def batch_body(b, oh):
            def chunk_body(c, carry):
                m, l, acc = carry
                t = (h * B + b) * nc + c

                @pl.when(t + nbuf - 1 < total)
                def _():
                    kv_start(t + nbuf - 1)

                slot = t % nbuf
                buf_wait(kbuf, ksem, slot)
                s = lax.dot_general(qh, kbuf[slot], (((1,), (1,)), ((), ())),
                                    preferred_element_type=_F32) * (DH ** -0.5)
                m_new = jnp.maximum(m, jnp.max(s, axis=-1, keepdims=True))
                alpha = jnp.exp(m - m_new)
                p = jnp.exp(s - m_new)
                l = alpha * l + jnp.sum(p, axis=-1, keepdims=True)
                buf_wait(vbuf, vsem, slot)
                acc = alpha * acc + jnp.dot(p.astype(_BF16), vbuf[slot],
                                            preferred_element_type=_F32)
                return m_new, l, acc

            m, l, acc = lax.fori_loop(
                0, nc, chunk_body,
                (jnp.full((B, 1), -jnp.inf, _F32), jnp.zeros((B, 1), _F32),
                 jnp.zeros((B, DH), _F32)))
            return jnp.where(row == b, acc / l, oh)

        oh = lax.fori_loop(0, B, batch_body, jnp.zeros((B, DH), _F32))
        wo_h = wo_v[:, pl.ds(pl.multiple_of(h * DH, DH), DH)]
        return attn + lax.dot_general(oh.astype(_BF16), wo_h, _NT,
                                      preferred_element_type=_F32)

    attn = lax.fori_loop(0, H, head_body, jnp.zeros((B, D), _F32))

    x1 = _r(x + _r(ga * _r(attn)))
    h2 = _r(_r(_r(_layernorm(x1)) * _r(1.0 + cb)) + sb)
    for i in range(5, 9):
        w_copy(i).wait()
    wr = wr_v[...].astype(_F32).reshape(1, D)
    r = _r(jnp.sum(h2 * wr, axis=-1, keepdims=True))
    hb = h2.astype(_BF16)
    g = _r(jnp.dot(hb, wg_v[...], preferred_element_type=_F32))
    g = _r(g * _r(jax.nn.sigmoid(g)))
    u = _r(jnp.dot(hb, wu_v[...], preferred_element_type=_F32))
    y = _r(lax.dot_general(_r(g * u).astype(_BF16), wd_v[...], _NT,
                           preferred_element_type=_F32))
    y = _r(y * _r(jax.nn.sigmoid(r)))
    moe = _r(h2 + _r(h2 * 0.0 + y))
    out_ref[...] = (x1 + _r(gb * moe)).astype(out_ref.dtype)


def _build(ch=2048, nbuf=4, sub=64, prio=(0, 1)):
    B, D, H, DH, F = _B, _D, _H, _DH, _F
    anyspec = pl.BlockSpec(memory_space=pltpu.HBM)
    return pl.pallas_call(
        functools.partial(_body, ch=ch, nbuf=nbuf, sub=sub, prio=prio),
        in_specs=[anyspec] * 11,
        out_specs=pl.BlockSpec(memory_space=pltpu.VMEM),
        out_shape=jax.ShapeDtypeStruct((B, D), _BF16),
        scratch_shapes=[
            pltpu.VMEM((B, D), _BF16),
            pltpu.VMEM((B, D), _BF16),
            pltpu.VMEM((D,), _BF16),
            pltpu.VMEM((D, 6 * D), _BF16),
            pltpu.VMEM((D, H * DH), _BF16),
            pltpu.VMEM((D, H * DH), _BF16),
            pltpu.VMEM((D, F), _BF16),
            pltpu.VMEM((D, F), _BF16),
            pltpu.VMEM((D, F), _BF16),
            pltpu.VMEM((nbuf, ch, DH), _BF16),
            pltpu.VMEM((nbuf, ch, DH), _BF16),
            pltpu.VMEM((B, H * DH), _F32),
            pltpu.SemaphoreType.DMA((9,)),
            pltpu.SemaphoreType.DMA((nbuf,)),
            pltpu.SemaphoreType.DMA((nbuf,)),
        ],
        compiler_params=pltpu.CompilerParams(
            vmem_limit_bytes=100 * 1024 * 1024),
    )


def _run(A_x, A_k_cache, A_v_cache, A_wq, A_wo, B_w_r, B_w_gate, B_w_up,
         B_w_down, c, w_mod, **cfg):
    out = _build(**cfg)(A_x.reshape(_B, _D), A_k_cache, A_v_cache, A_wq, A_wo.T,
                        B_w_r, B_w_gate, B_w_up, B_w_down.T, c, w_mod)
    return out.reshape(_B, 1, _D)


@jax.jit
def pallas_adaLN_cond__mha_block_cached__moe_arch_mod__decode_kernel(
    A_x, A_k_cache, A_v_cache, A_wq, A_wo, B_x, B_w_r, B_w_gate, B_w_up,
    B_w_down, c, w_mod,
):
    del B_x
    return _run(A_x, A_k_cache, A_v_cache, A_wq, A_wo, B_w_r, B_w_gate, B_w_up,
                B_w_down, c, w_mod)
```

```python
import functools

import jax
import jax.numpy as jnp
from jax import lax
import jax.experimental.pallas as pl
import jax.experimental.pallas.tpu as pltpu

_B, _D, _H, _DH, _SK, _F = 4, 448, 16, 256, 16384, 1792
_F32, _BF16 = jnp.float32, jnp.bfloat16
_NT = (((1,), (1,)), ((), ()))


def _layernorm(x):
    m = jnp.mean(x, axis=-1, keepdims=True)
    d = x - m
    v = jnp.mean(d * d, axis=-1, keepdims=True)
    return d / jnp.sqrt(v + 1e-5)


def _r(x):
    return x.astype(_BF16).astype(_F32)


def _body(x_hbm, k_hbm, v_hbm, wq_hbm, wo_hbm, wr_hbm, wg_hbm, wu_hbm, wd_hbm,
          c_hbm, wm_hbm, out_ref,
          x_v, c_v, wr_v, wm_v, wq_v, wo_v, wg_v, wu_v, wd_v,
          kbuf, vbuf, q_v, wsem, ksem, vsem, *, ch, nbuf, sub, prio):
    B, D, H, DH = _B, _D, _H, _DH
    nc = _SK // ch
    total = H * B * nc

    def w_copy(i):
        src, dst = ((c_hbm, c_v), (wm_hbm, wm_v), (x_hbm, x_v), (wq_hbm, wq_v),
                    (wo_hbm, wo_v), (wr_hbm, wr_v), (wg_hbm, wg_v),
                    (wu_hbm, wu_v), (wd_hbm, wd_v))[i]
        return pltpu.make_async_copy(src, dst, wsem.at[i])

    def kv_start(t):
        h = t // (B * nc)
        b = (t // nc) % B
        slot = t % nbuf
        base = (t % nc) * ch
        n = 0
        for o in range(0, ch, sub):
            sz = min(sub, ch - o)
            off = pl.multiple_of(base + o, 16)
            for src, dst, sem in ((k_hbm, kbuf, ksem), (v_hbm, vbuf, vsem)):
                pltpu.make_async_copy(
                    src.at[b, h, pl.ds(off, sz), :],
                    dst.at[slot, pl.ds(o, sz), :],
                    sem.at[slot]).start(priority=prio[n % len(prio)])
                n += 1

    def buf_wait(buf, sem, slot):
        pltpu.make_async_copy(buf.at[slot], buf.at[slot], sem.at[slot]).wait()

    for i in range(4):
        w_copy(i).start()
    for t in range(nbuf - 1):
        kv_start(t)
    for i in range(4, 9):
        w_copy(i).start()

    w_copy(0).wait()
    w_copy(1).wait()
    cc = c_v[...].astype(_F32)
    sc = _r(cc * _r(jax.nn.sigmoid(cc)))
    mod = _r(jnp.dot(sc.astype(_BF16), wm_v[...], preferred_element_type=_F32))
    sa, ca, ga, sb, cb, gb = (mod[:, i * D:(i + 1) * D] for i in range(6))

    w_copy(2).wait()
    x = x_v[...].astype(_F32)
    h1 = _r(_r(_r(_layernorm(x)) * _r(1.0 + ca)) + sa)
    w_copy(3).wait()
    q = _r(jnp.dot(h1.astype(_BF16), wq_v[...], preferred_element_type=_F32))
    q_v[...] = q

    w_copy(4).wait()
    row = lax.broadcasted_iota(jnp.int32, (B, DH), 0)

    def head_body(h, attn):
        qh = q_v[:, pl.ds(pl.multiple_of(h * DH, DH), DH)].astype(_BF16)

        def batch_body(b, oh):
            def chunk_body(c, carry):
                m, l, acc = carry
                t = (h * B + b) * nc + c

                @pl.when(t + nbuf - 1 < total)
                def _():
                    kv_start(t + nbuf - 1)

                slot = t % nbuf
                buf_wait(kbuf, ksem, slot)
                s = lax.dot_general(qh, kbuf[slot], (((1,), (1,)), ((), ())),
                                    preferred_element_type=_F32) * (DH ** -0.5)
                m_new = jnp.maximum(m, jnp.max(s, axis=-1, keepdims=True))
                alpha = jnp.exp(m - m_new)
                p = jnp.exp(s - m_new)
                l = alpha * l + jnp.sum(p, axis=-1, keepdims=True)
                buf_wait(vbuf, vsem, slot)
                acc = alpha * acc + jnp.dot(p.astype(_BF16), vbuf[slot],
                                            preferred_element_type=_F32)
                return m_new, l, acc

            m, l, acc = lax.fori_loop(
                0, nc, chunk_body,
                (jnp.full((B, 1), -jnp.inf, _F32), jnp.zeros((B, 1), _F32),
                 jnp.zeros((B, DH), _F32)))
            return jnp.where(row == b, acc / l, oh)

        oh = lax.fori_loop(0, B, batch_body, jnp.zeros((B, DH), _F32))
        wo_h = wo_v[:, pl.ds(pl.multiple_of(h * DH, DH), DH)]
        return attn + lax.dot_general(oh.astype(_BF16), wo_h, _NT,
                                      preferred_element_type=_F32)

    attn = lax.fori_loop(0, H, head_body, jnp.zeros((B, D), _F32))

    x1 = _r(x + _r(ga * _r(attn)))
    h2 = _r(_r(_r(_layernorm(x1)) * _r(1.0 + cb)) + sb)
    for i in range(5, 9):
        w_copy(i).wait()
    wr = wr_v[...].astype(_F32).reshape(1, D)
    r = _r(jnp.sum(h2 * wr, axis=-1, keepdims=True))
    hb = h2.astype(_BF16)
    g = _r(jnp.dot(hb, wg_v[...], preferred_element_type=_F32))
    g = _r(g * _r(jax.nn.sigmoid(g)))
    u = _r(jnp.dot(hb, wu_v[...], preferred_element_type=_F32))
    y = _r(lax.dot_general(_r(g * u).astype(_BF16), wd_v[...], _NT,
                           preferred_element_type=_F32))
    y = _r(y * _r(jax.nn.sigmoid(r)))
    moe = _r(h2 + _r(h2 * 0.0 + y))
    out_ref[...] = (x1 + _r(gb * moe)).astype(out_ref.dtype)


def _build(ch=1024, nbuf=6, sub=96, prio=(0, 1, 1, 0), interpret=False):
    B, D, H, DH, F = _B, _D, _H, _DH, _F
    anyspec = pl.BlockSpec(memory_space=pltpu.HBM)
    return pl.pallas_call(
        functools.partial(_body, ch=ch, nbuf=nbuf, sub=sub, prio=prio),
        in_specs=[anyspec] * 11,
        out_specs=pl.BlockSpec(memory_space=pltpu.VMEM),
        out_shape=jax.ShapeDtypeStruct((B, D), _BF16),
        scratch_shapes=[
            pltpu.VMEM((B, D), _BF16),
            pltpu.VMEM((B, D), _BF16),
            pltpu.VMEM((D,), _BF16),
            pltpu.VMEM((D, 6 * D), _BF16),
            pltpu.VMEM((D, H * DH), _BF16),
            pltpu.VMEM((D, H * DH), _BF16),
            pltpu.VMEM((D, F), _BF16),
            pltpu.VMEM((D, F), _BF16),
            pltpu.VMEM((D, F), _BF16),
            pltpu.VMEM((nbuf, ch, DH), _BF16),
            pltpu.VMEM((nbuf, ch, DH), _BF16),
            pltpu.VMEM((B, H * DH), _F32),
            pltpu.SemaphoreType.DMA((9,)),
            pltpu.SemaphoreType.DMA((nbuf,)),
            pltpu.SemaphoreType.DMA((nbuf,)),
        ],
        compiler_params=pltpu.CompilerParams(
            vmem_limit_bytes=100 * 1024 * 1024),
        interpret=interpret,
    )


def _run(A_x, A_k_cache, A_v_cache, A_wq, A_wo, B_w_r, B_w_gate, B_w_up,
         B_w_down, c, w_mod, **cfg):
    out = _build(**cfg)(A_x.reshape(_B, _D), A_k_cache, A_v_cache, A_wq, A_wo.T,
                        B_w_r, B_w_gate, B_w_up, B_w_down.T, c, w_mod)
    return out.reshape(_B, 1, _D)


@jax.jit
def pallas_adaLN_cond__mha_block_cached__moe_arch_mod__decode_kernel(
    A_x, A_k_cache, A_v_cache, A_wq, A_wo, B_x, B_w_r, B_w_gate, B_w_up,
    B_w_down, c, w_mod,
):
    del B_x
    return _run(A_x, A_k_cache, A_v_cache, A_wq, A_wo, B_w_r, B_w_gate, B_w_up,
                B_w_down, c, w_mod)
```

```python
import functools

import jax
import jax.numpy as jnp
from jax import lax
import jax.experimental.pallas as pl
import jax.experimental.pallas.tpu as pltpu

_B, _D, _H, _DH, _SK, _F = 4, 448, 16, 256, 16384, 1792
_F32, _BF16 = jnp.float32, jnp.bfloat16
_NT = (((1,), (1,)), ((), ()))


def _layernorm(x):
    m = jnp.mean(x, axis=-1, keepdims=True)
    d = x - m
    v = jnp.mean(d * d, axis=-1, keepdims=True)
    return d / jnp.sqrt(v + 1e-5)


def _r(x):
    return x.astype(_BF16).astype(_F32)


def _body(x_hbm, k_hbm, v_hbm, wq_hbm, wo_hbm, wr_hbm, wg_hbm, wu_hbm, wd_hbm,
          c_hbm, wm_hbm, out_ref,
          x_v, c_v, wr_v, wm_v, wq_v, wo_v, wg_v, wu_v, wd_v,
          kbuf, vbuf, q_v, wsem, ksem, vsem, *, ch, nbuf, sub, prio, vrot, wrows):
    B, D, H, DH = _B, _D, _H, _DH
    nc = _SK // ch
    total = H * B * nc

    def w_copy(i):
        src, dst = ((c_hbm, c_v), (wm_hbm, wm_v), (x_hbm, x_v), (wq_hbm, wq_v),
                    (wo_hbm, wo_v), (wr_hbm, wr_v), (wg_hbm, wg_v),
                    (wu_hbm, wu_v), (wd_hbm, wd_v))[i]
        return pltpu.make_async_copy(src, dst, wsem.at[i])

    def w_start(i):
        src, dst = ((c_hbm, c_v), (wm_hbm, wm_v), (x_hbm, x_v), (wq_hbm, wq_v),
                    (wo_hbm, wo_v), (wr_hbm, wr_v), (wg_hbm, wg_v),
                    (wu_hbm, wu_v), (wd_hbm, wd_v))[i]
        if dst.shape[0] != D or len(dst.shape) != 2 or not wrows:
            w_copy(i).start()
            return
        for n, o in enumerate(range(0, D, wrows)):
            pltpu.make_async_copy(src.at[pl.ds(o, wrows), :],
                                  dst.at[pl.ds(o, wrows), :],
                                  wsem.at[i]).start(priority=n % 2)

    def kv_start(t):
        h = t // (B * nc)
        b = (t // nc) % B
        slot = t % nbuf
        base = (t % nc) * ch
        pieces, o, i = [], 0, 0
        while o < ch:
            sz = min(sub[i % len(sub)], ch - o)
            pieces.append((o, sz))
            o, i = o + sz, i + 1
        n = 0
        for i in range(len(pieces)):
            for src, dst, sem, rot in ((k_hbm, kbuf, ksem, 0),
                                       (v_hbm, vbuf, vsem, vrot)):
                o, sz = pieces[(i + rot) % len(pieces)]
                pltpu.make_async_copy(
                    src.at[b, h, pl.ds(pl.multiple_of(base + o, 16), sz), :],
                    dst.at[slot, pl.ds(o, sz), :],
                    sem.at[slot]).start(priority=prio[n % len(prio)])
                n += 1

    def buf_wait(buf, sem, slot):
        pltpu.make_async_copy(buf.at[slot], buf.at[slot], sem.at[slot]).wait()

    for i in range(4):
        w_start(i)
    for t in range(nbuf - 1):
        kv_start(t)
    for i in range(4, 9):
        w_start(i)

    w_copy(0).wait()
    w_copy(1).wait()
    cc = c_v[...].astype(_F32)
    sc = _r(cc * _r(jax.nn.sigmoid(cc)))
    mod = _r(jnp.dot(sc.astype(_BF16), wm_v[...], preferred_element_type=_F32))
    sa, ca, ga, sb, cb, gb = (mod[:, i * D:(i + 1) * D] for i in range(6))

    w_copy(2).wait()
    x = x_v[...].astype(_F32)
    h1 = _r(_r(_r(_layernorm(x)) * _r(1.0 + ca)) + sa)
    w_copy(3).wait()
    q = _r(jnp.dot(h1.astype(_BF16), wq_v[...], preferred_element_type=_F32))
    q_v[...] = q

    row = lax.broadcasted_iota(jnp.int32, (B, DH), 0)

    def head_body(h, attn):
        qh = q_v[:, pl.ds(pl.multiple_of(h * DH, DH), DH)].astype(_BF16)

        def batch_body(b, oh):
            def chunk_body(c, carry):
                m, l, acc = carry
                t = (h * B + b) * nc + c

                @pl.when(t + nbuf - 1 < total)
                def _():
                    kv_start(t + nbuf - 1)

                slot = t % nbuf
                buf_wait(kbuf, ksem, slot)
                s = lax.dot_general(qh, kbuf[slot], (((1,), (1,)), ((), ())),
                                    preferred_element_type=_F32) * (DH ** -0.5)
                m_new = jnp.maximum(m, jnp.max(s, axis=-1, keepdims=True))
                alpha = jnp.exp(m - m_new)
                p = jnp.exp(s - m_new)
                l = alpha * l + jnp.sum(p, axis=-1, keepdims=True)
                buf_wait(vbuf, vsem, slot)
                acc = alpha * acc + jnp.dot(p.astype(_BF16), vbuf[slot],
                                            preferred_element_type=_F32)
                return m_new, l, acc

            m, l, acc = lax.fori_loop(
                0, nc, chunk_body,
                (jnp.full((B, 1), -jnp.inf, _F32), jnp.zeros((B, 1), _F32),
                 jnp.zeros((B, DH), _F32)))
            return jnp.where(row == b, acc / l, oh)

        oh = lax.fori_loop(0, B, batch_body, jnp.zeros((B, DH), _F32))

        @pl.when(h == 0)
        def _():
            w_copy(4).wait()

        wo_h = wo_v[:, pl.ds(pl.multiple_of(h * DH, DH), DH)]
        return attn + lax.dot_general(oh.astype(_BF16), wo_h, _NT,
                                      preferred_element_type=_F32)

    attn = lax.fori_loop(0, H, head_body, jnp.zeros((B, D), _F32))

    x1 = _r(x + _r(ga * _r(attn)))
    h2 = _r(_r(_r(_layernorm(x1)) * _r(1.0 + cb)) + sb)
    for i in range(5, 9):
        w_copy(i).wait()
    wr = wr_v[...].astype(_F32).reshape(1, D)
    r = _r(jnp.sum(h2 * wr, axis=-1, keepdims=True))
    hb = h2.astype(_BF16)
    g = _r(jnp.dot(hb, wg_v[...], preferred_element_type=_F32))
    g = _r(g * _r(jax.nn.sigmoid(g)))
    u = _r(jnp.dot(hb, wu_v[...], preferred_element_type=_F32))
    y = _r(lax.dot_general(_r(g * u).astype(_BF16), wd_v[...], _NT,
                           preferred_element_type=_F32))
    y = _r(y * _r(jax.nn.sigmoid(r)))
    moe = _r(h2 + _r(h2 * 0.0 + y))
    out_ref[...] = (x1 + _r(gb * moe)).astype(out_ref.dtype)


def _build(ch=1024, nbuf=6, sub=(96,), vrot=3, wrows=16, prio=(0, 1, 1, 0), interpret=False):
    B, D, H, DH, F = _B, _D, _H, _DH, _F
    anyspec = pl.BlockSpec(memory_space=pltpu.HBM)
    return pl.pallas_call(
        functools.partial(_body, ch=ch, nbuf=nbuf, sub=sub, prio=prio, vrot=vrot, wrows=wrows),
        in_specs=[anyspec] * 11,
        out_specs=pl.BlockSpec(memory_space=pltpu.VMEM),
        out_shape=jax.ShapeDtypeStruct((B, D), _BF16),
        scratch_shapes=[
            pltpu.VMEM((B, D), _BF16),
            pltpu.VMEM((B, D), _BF16),
            pltpu.VMEM((D,), _BF16),
            pltpu.VMEM((D, 6 * D), _BF16),
            pltpu.VMEM((D, H * DH), _BF16),
            pltpu.VMEM((D, H * DH), _BF16),
            pltpu.VMEM((D, F), _BF16),
            pltpu.VMEM((D, F), _BF16),
            pltpu.VMEM((D, F), _BF16),
            pltpu.VMEM((nbuf, ch, DH), _BF16),
            pltpu.VMEM((nbuf, ch, DH), _BF16),
            pltpu.VMEM((B, H * DH), _F32),
            pltpu.SemaphoreType.DMA((9,)),
            pltpu.SemaphoreType.DMA((nbuf,)),
            pltpu.SemaphoreType.DMA((nbuf,)),
        ],
        compiler_params=pltpu.CompilerParams(
            vmem_limit_bytes=100 * 1024 * 1024),
        interpret=interpret,
    )


def _run(A_x, A_k_cache, A_v_cache, A_wq, A_wo, B_w_r, B_w_gate, B_w_up,
         B_w_down, c, w_mod, **cfg):
    out = _build(**cfg)(A_x.reshape(_B, _D), A_k_cache, A_v_cache, A_wq, A_wo.T,
                        B_w_r, B_w_gate, B_w_up, B_w_down.T, c, w_mod)
    return out.reshape(_B, 1, _D)


@jax.jit
def pallas_adaLN_cond__mha_block_cached__moe_arch_mod__decode_kernel(
    A_x, A_k_cache, A_v_cache, A_wq, A_wo, B_x, B_w_r, B_w_gate, B_w_up,
    B_w_down, c, w_mod,
):
    del B_x
    return _run(A_x, A_k_cache, A_v_cache, A_wq, A_wo, B_w_r, B_w_gate, B_w_up,
                B_w_down, c, w_mod)
```
